```python
import os as _os
_os.environ.setdefault("JAX_PLATFORMS", "cpu")
import jax
import jax.numpy as jnp

def _softmax(x, axis=-1):
    return jax.nn.softmax(x, axis=axis)
def _gelu(x):
    return jax.nn.gelu(x, approximate=True)
def _silu(x):
    return jax.nn.silu(x)
def _sigmoid(x):
    return jax.nn.sigmoid(x)
def _layernorm(x, axis=-1, eps=1e-5):
    m = jnp.mean(x, axis=axis, keepdims=True)
    v = jnp.var(x, axis=axis, keepdims=True)
    return (x - m) / jnp.sqrt(v + eps)
def _scatter_add(tgt, idx, src, axis=0):
    return tgt.at[idx].add(src)
def _segment_sum(src, seg, n):
    return jax.ops.segment_sum(src, seg, n)
class _Rng:
    def __init__(self, key):
        self._k = key
    def _next(self):
        self._k, sub = jax.random.split(self._k)
        return sub
    def normal(self, shape):
        return jax.random.normal(self._next(), shape, dtype=jnp.bfloat16)
    def randint(self, lo, hi, shape):
        return jax.random.randint(self._next(), shape, lo, hi, dtype=jnp.int32)
    def uniform(self, shape, lo=0.0, hi=1.0):
        return jax.random.uniform(self._next(), shape, jnp.bfloat16, lo, hi)
    def permutation(self, n):
        return jax.random.permutation(self._next(), n)


kernel_name = 'gated_mix__sliding_block_cached__mha_block_cached__decode'

def setup_inputs():
    _rng = _Rng(jax.random.key(int.from_bytes(__import__("os").urandom(4), "little")))
    _w = (lambda a: (lambda t: t.astype(jnp.bfloat16) if jnp.issubdtype(t.dtype, jnp.floating) else t)(jnp.asarray(a)))
    def _A_setup():
        B, Sq, D = 2, 1, 640
        Hq, Hkv, Sk, Dh = 32, 32, 4096, 128
        assert Hq % Hkv == 0, (Hq, Hkv)
        return {
            "x": _w((lambda *s: _rng.normal(s) * 0.05)(B, Sq, D)),
            "k_cache": _w((lambda *s: _rng.normal(s) * 3.2)(B, Hkv, Sk, Dh)),
            "v_cache": _w((lambda *s: _rng.normal(s) * 0.05)(B, Hkv, Sk, Dh)),
            "wq": _w((lambda *s: _rng.normal(s) * 3.2)(D, Hq * Dh) * (D ** -0.5)),
            "wo": _w((lambda *s: _rng.normal(s) * 0.05)(Hq * Dh, D) * ((Hq * Dh) ** -0.5)),
        }
    _A_in = _A_setup()

    def _B_setup():
        B, Sq, D = 2, 1, 640
        H, Sk, Dh = 32, 4096, 128
        return {
            "x": _w((lambda *s: _rng.normal(s) * 0.05)(B, Sq, D)),
            "k_cache": _w((lambda *s: _rng.normal(s) * 3.2)(B, H, Sk, Dh)),
            "v_cache": _w((lambda *s: _rng.normal(s) * 0.05)(B, H, Sk, Dh)),
            "wq": _w((lambda *s: _rng.normal(s) * 3.2)(D, H * Dh) * (D ** -0.5)),
            "wo": _w((lambda *s: _rng.normal(s) * 0.05)(H * Dh, D) * ((H * Dh) ** -0.5)),
        }
    _B_in = _B_setup()

    return {
        "A_x": _A_in["x"],
        "A_k_cache": _A_in["k_cache"],
        "A_v_cache": _A_in["v_cache"],
        "A_wq": _A_in["wq"],
        "A_wo": _A_in["wo"],
        "B_x": _B_in["x"],
        "B_k_cache": _B_in["k_cache"],
        "B_v_cache": _B_in["v_cache"],
        "B_wq": _B_in["wq"],
        "B_wo": _B_in["wo"],
        "gate_w": _w((lambda *s: _rng.normal(s) * 0.05)(640) * 16.0),
    }

def reference(A_x, A_k_cache, A_v_cache, A_wq, A_wo, B_x, B_k_cache, B_v_cache, B_wq, B_wo, gate_w):
    def _A_ref(x, k_cache, v_cache, wq, wo):
        B, Sq, D = x.shape
        Hq, Dh = 32, 128
        Hkv, Sk = k_cache.shape[1], k_cache.shape[2]
        W = min(4096, max(256, Sk // 4))
        rep = Hq // Hkv
        q = (lambda x, *d: x.transpose(*d))((x @ wq).reshape(B, Sq, Hq, Dh), 0, 2, 1, 3)
        k = jnp.repeat(k_cache[:, :, Sk - W:, :], rep, axis=1)
        v = jnp.repeat(v_cache[:, :, Sk - W:, :], rep, axis=1)
        scores = jnp.einsum("bhqd,bhkd->bhqk", q, k) * (Dh ** -0.5)
        p = _softmax(scores, axis=-1)
        o = jnp.einsum("bhqk,bhkd->bhqd", p, v)
        return (lambda x, *d: x.transpose(*d))(o, 0, 2, 1, 3).reshape(B, Sq, Hq * Dh) @ wo

    def _B_ref(x, k_cache, v_cache, wq, wo):
        B, Sq, D = x.shape
        H, Dh = 32, 128
        q = (lambda x, *d: x.transpose(*d))((x @ wq).reshape(B, Sq, H, Dh), 0, 2, 1, 3)
        scores = jnp.einsum("bhqd,bhkd->bhqk", q, k_cache) * (Dh ** -0.5)
        p = _softmax(scores, axis=-1)
        o = jnp.einsum("bhqk,bhkd->bhqd", p, v_cache)
        return (lambda x, *d: x.transpose(*d))(o, 0, 2, 1, 3).reshape(B, Sq, H * Dh) @ wo

    x = A_x
    g = _sigmoid((x * gate_w).sum(-1, keepdims=True))
    a = _A_ref(x, A_k_cache, A_v_cache, A_wq, A_wo)
    b = _B_ref(x, B_k_cache, B_v_cache, B_wq, B_wo)
    return g * a + (1 - g) * b
```

```python
import functools
import jax
import jax.numpy as jnp
from jax import lax
from jax.experimental import pallas as pl
from jax.experimental.pallas import tpu as pltpu

B, D, H, DH, SK = 2, 640, 32, 128, 4096
WIN = min(4096, max(256, SK // 4))
NG = 8
PR = 64
SCALE = DH ** -0.5
NT = (((1,), (1,)), ((), ()))


def _bits(t, order):
    out = {}
    for i, (name, bit) in enumerate(order):
        out[name] = out.get(name, 0) + (((t >> i) & 1) << bit)
    return out


def make(order_b=(("b", 0), ("hh", 0), ("s", 3), ("s", 0), ("s", 1), ("s", 2), ("s", 4), ("s", 5)),
         order_a=(("b", 0), ("hh", 0), ("s", 3), ("s", 0), ("s", 1), ("s", 2)),
         compute=True, nslot=3, wo_rows=32, a_pos="end", flags=None):

    def kernel(x_hbm, gw_hbm, ak, av, awq, awo, bk, bv, bwq, bwo, o_ref,
               x_v, gw_v, wq_v, wo_v, bbuf, abuf, q_scr, sb_scr, sa_scr, pb_scr, pa_scr, o_scr,
               sem_small, sem_wq, sem_wo, sem_kv):
        row = lax.broadcasted_iota(jnp.int32, (8, DH), 0)

        def issue_kv(src_b, src_a, g, j, slot):
            def one(src, dst, order, nu, u, base):
                f = _bits(u, order[:nu])
                fj = _bits(j, order[nu:])
                b = f.get("b", 0) + fj.get("b", 0)
                hh = f.get("hh", 0) + fj.get("hh", 0)
                s = f.get("s", 0) + fj.get("s", 0)
                r0 = pl.multiple_of(s * PR, PR)
                pltpu.make_async_copy(
                    src.at[b, pl.ds(2 * g + 16 * hh, 2), pl.ds(base + r0, PR), :],
                    dst.at[slot, pl.ds(4 * b + 2 * hh, 2), pl.ds(r0, PR), :],
                    sem_kv.at[slot]).start(priority=u & 1)
            if a_pos == "end":
                for u in range(32):
                    one(src_b, bbuf, order_b, 5, u, 0)
                for u in range(8):
                    one(src_a, abuf, order_a, 3, u, SK - WIN)
            else:
                for u in range(32):
                    one(src_b, bbuf, order_b, 5, u, 0)
                    if u % 8 == 7:
                        for uu in range(2):
                            one(src_a, abuf, order_a, 3, (u // 8) * 2 + uu, SK - WIN)

        def wait_kv(slot):
            pltpu.make_async_copy(bbuf.at[slot], bbuf.at[slot], sem_kv.at[slot]).wait()
            pltpu.make_async_copy(abuf.at[slot], abuf.at[slot], sem_kv.at[slot]).wait()

        def issue_wq(i, _):
            r0 = pl.multiple_of(i * 16, 16)
            for c in range(4):
                for m, w in enumerate((awq, bwq)):
                    pltpu.make_async_copy(w.at[pl.ds(r0, 16), pl.ds(c * 1024, 1024)],
                                          wq_v.at[m, pl.ds(r0, 16), pl.ds(c * 1024, 1024)],
                                          sem_wq).start(priority=m)
        issue_wq(0, None)
        cx = pltpu.make_async_copy(x_hbm, x_v, sem_small.at[0])
        cg = pltpu.make_async_copy(gw_hbm, gw_v, sem_small.at[1])
        cx.start()
        cg.start()
        lax.fori_loop(1, D // 16, issue_wq, None)

        def first_k(j, _):
            issue_kv(bk, ak, 0, j, 0)
        lax.fori_loop(0, 2, first_k, None)
        cx.wait()
        cg.wait()
        pltpu.make_async_copy(wq_v, wq_v, sem_wq).wait()

        xf = x_v[...].astype(jnp.float32)
        row_d = lax.broadcasted_iota(jnp.int32, (8, D), 0)
        x8 = jnp.where(row_d < 4, xf[0:1, :], xf[1:2, :]).astype(jnp.bfloat16)

        def qproj(j, _):
            issue_kv(bk, ak, 0, j + 2, 0)
            if compute:
                for m in range(2):
                    c0 = pl.multiple_of(j * 1024, 1024)
                    r = jnp.dot(x8, wq_v[m, :, pl.ds(c0, 1024)], preferred_element_type=jnp.float32)
                    for hh in range(8):
                        q_scr[m, j * 8 + hh] = r[:, hh * DH:(hh + 1) * DH]
        lax.fori_loop(0, 4, qproj, None)

        def rest_k(j, _):
            issue_kv(bk, ak, 0, j, 0)
        lax.fori_loop(6, 8, rest_k, None)
        issue_kv(bv, av, 0, 0, 1)

        def head_of(g, j):
            return 2 * g + (j & 1) + 16 * ((j >> 1) & 1)

        def qk_step(g, j, slot):
            h = head_of(g, j)
            for m, (buf, scr, n) in enumerate(((bbuf, sb_scr, SK), (abuf, sa_scr, WIN))):
                q = q_scr[1 - m, h].astype(jnp.bfloat16)
                s = lax.dot_general(q, buf[slot, j], NT, preferred_element_type=jnp.float32)
                rown = lax.broadcasted_iota(jnp.int32, (8, n), 0)
                pltpu.store(scr, s, mask=rown == j)

        def softmax():
            ls = []
            for scr, p_scr in ((sb_scr, pb_scr), (sa_scr, pa_scr)):
                s = scr[...] * SCALE
                e = jnp.exp(s - jnp.max(s, axis=-1, keepdims=True))
                ls.append(jnp.sum(e, axis=-1, keepdims=True))
                p_scr[...] = e.astype(jnp.bfloat16)
            return ls

        def pv_step(j, slot, ob, oa):
            rb = jnp.dot(pb_scr[...], bbuf[slot, j], preferred_element_type=jnp.float32)
            ra = jnp.dot(pa_scr[...], abuf[slot, j], preferred_element_type=jnp.float32)
            return jnp.where(row == j, rb, ob), jnp.where(row == j, ra, oa)

        n_wo = (H * DH) // wo_rows // 8

        def issue_wo(j):
            for u in range(n_wo):
                r0 = pl.multiple_of(j * (H * DH // 8) + u * wo_rows, wo_rows)
                for m, w in enumerate((awo, bwo)):
                    pltpu.make_async_copy(w.at[pl.ds(r0, wo_rows), :], wo_v.at[m, pl.ds(r0, wo_rows), :],
                                          sem_wo.at[j]).start(priority=m)

        sb_scr[...] = jnp.zeros_like(sb_scr)
        sa_scr[...] = jnp.zeros_like(sa_scr)
        o_scr[...] = jnp.zeros_like(o_scr)

        def group(g, _):
            ks = (2 * g) % nslot
            vs = (2 * g + 1) % nslot
            kn = (2 * g + 2) % nslot
            vn = (2 * g + 3) % nslot
            last = g == NG - 1

            def qk(j, _):
                @pl.when(j < 7)
                def _():
                    issue_kv(bv, av, g, j + 1, vs)

                @pl.when(jnp.logical_and(j == 7, jnp.logical_not(last)))
                def _():
                    issue_kv(bk, ak, g + 1, 0, kn)

                @pl.when(jnp.logical_and(j == 7, last))
                def _():
                    issue_wo(0)

                @pl.when(j == 0)
                def _():
                    wait_kv(ks)
                if compute:
                    qk_step(g, j, ks)
            lax.fori_loop(0, 8, qk, None)
            if compute:
                lb, la = softmax()

            def pv(j, carry):
                @pl.when(jnp.logical_and(j < 7, jnp.logical_not(last)))
                def _():
                    issue_kv(bk, ak, g + 1, j + 1, kn)

                @pl.when(jnp.logical_and(j == 7, jnp.logical_not(last)))
                def _():
                    issue_kv(bv, av, g + 1, 0, vn)

                @pl.when(jnp.logical_and(j < 7, last))
                def _():
                    issue_wo(j + 1)

                @pl.when(j == 0)
                def _():
                    wait_kv(vs)
                if compute:
                    return pv_step(j, vs, *carry)
                return carry
            z = jnp.zeros((8, DH), jnp.float32)
            ob, oa = lax.fori_loop(0, 8, pv, (z, z))
            if compute:
                for m, o in ((0, oa / la), (1, ob / lb)):
                    for r in range(8):
                        h = head_of(g, r)
                        o_scr[m, h, pl.ds(r // 4, 1), :] = o[r:r + 1, :]
        lax.fori_loop(0, NG, group, None)

        def proj(j, acc):
            pltpu.make_async_copy(wo_v.at[:, pl.ds(0, H * DH // 8), :], wo_v.at[:, pl.ds(0, H * DH // 8), :], sem_wo.at[j]).wait()
            if not compute:
                return acc
            out = []
            for m in range(2):
                lhs = jnp.concatenate([o_scr[m, 4 * j + i] for i in range(4)], axis=1).astype(jnp.bfloat16)
                r0 = pl.multiple_of(j * 512, 512)
                out.append(acc[m] + jnp.dot(lhs, wo_v[m, pl.ds(r0, 512), :], preferred_element_type=jnp.float32))
            return tuple(out)
        z = jnp.zeros((8, D), jnp.float32)
        gw = gw_v[...].astype(jnp.float32)
        logit = sum(jnp.sum(xf[:, c * DH:(c + 1) * DH] * gw[c:c + 1, :], axis=-1, keepdims=True) for c in range(D // DH))
        gate = jax.nn.sigmoid(logit)
        acc_a, acc_b = lax.fori_loop(0, 8, proj, (z, z))
        o_ref[...] = (gate * acc_a[0:2] + (1.0 - gate) * acc_b[0:2]).astype(o_ref.dtype)

    def fn(A_x, A_k, A_v, A_wq, A_wo, B_x, B_k, B_v, B_wq, B_wo, gate_w):
        hbm = pl.BlockSpec(memory_space=pltpu.HBM)
        out = pl.pallas_call(
            kernel,
            in_specs=[hbm] * 10,
            out_specs=pl.BlockSpec(memory_space=pltpu.VMEM),
            out_shape=jax.ShapeDtypeStruct((B, D), jnp.bfloat16),
            scratch_shapes=[
                pltpu.VMEM((B, D), jnp.bfloat16),
                pltpu.VMEM((D // DH, DH), jnp.bfloat16),
                pltpu.VMEM((2, D, H * DH), jnp.bfloat16),
                pltpu.VMEM((2, H * DH, D), jnp.bfloat16),
                pltpu.VMEM((nslot, 8, SK, DH), jnp.bfloat16),
                pltpu.VMEM((nslot, 8, WIN, DH), jnp.bfloat16),
                pltpu.VMEM((2, H, 8, DH), jnp.float32),
                pltpu.VMEM((8, SK), jnp.float32),
                pltpu.VMEM((8, WIN), jnp.float32),
                pltpu.VMEM((8, SK), jnp.bfloat16),
                pltpu.VMEM((8, WIN), jnp.bfloat16),
                pltpu.VMEM((2, H, 8, DH), jnp.float32),
                pltpu.SemaphoreType.DMA((2,)),
                pltpu.SemaphoreType.DMA(()),
                pltpu.SemaphoreType.DMA((8,)),
                pltpu.SemaphoreType.DMA((nslot,)),
            ],
            compiler_params=pltpu.CompilerParams(vmem_limit_bytes=100 * 2**20, disable_bounds_checks=True, flags=flags),
        )(A_x.reshape(B, D), gate_w.reshape(D // DH, DH), A_k, A_v, A_wq, A_wo, B_k, B_v, B_wq, B_wo)
        return out.reshape(B, 1, D)
    return fn


_impl = make(a_pos="mix")


@jax.jit
def pallas_gated_mix__sliding_block_cached__mha_block_cached__decode_kernel(
    A_x, A_k_cache, A_v_cache, A_wq, A_wo, B_x, B_k_cache, B_v_cache, B_wq, B_wo, gate_w,
):
    return _impl(A_x, A_k_cache, A_v_cache, A_wq, A_wo, B_x, B_k_cache, B_v_cache, B_wq, B_wo, gate_w)
```

```python
import jax
import jax.numpy as jnp
from jax import lax
from jax.experimental import pallas as pl
from jax.experimental.pallas import tpu as pltpu

B, D, H, DH, SK = 2, 640, 32, 128, 4096
WIN = min(4096, max(256, SK // 4))
SCALE = DH**-0.5

OCT = 8
N_OCT = H // OCT
N_GROUP = B * N_OCT // 2
KU = WIN
NB = SK // KU
NU = NB + 1
SPU = 4
PASS = NU * SPU
N_STEP = N_GROUP * 2 * PASS
PIECE = 64
PPU = KU // PIECE
SKEW = 6
AHEAD = 7
N_SLOT = 6
WQ_SEG = 5
WO_ROWS = 32

_NT = (((1,), (1,)), ((), ()))


def _kernel(
    x_hbm, gw_hbm, ak_hbm, av_hbm, awq_hbm, awo_hbm, bk_hbm, bv_hbm, bwq_hbm, bwo_hbm,
    out_ref,
    x_v, gw_v, wq_v, wo_v, kv_v, q_scr, s_scr, p_scr, l_scr, acc_scr, o_scr,
    sem_small, sem_wq, sem_wo, sem_kv,
):
    row = lax.broadcasted_iota(jnp.int32, (OCT, DH), 0)

    def wait_all(buf, sem):
        pltpu.make_async_copy(buf, buf, sem).wait()

    def issue_wq(k, _):
        r0 = pl.multiple_of((k // 4) * 8, 8)
        c0 = pl.multiple_of((k % 4) * 1024, 1024)
        for lo, n in ((0, 2), (2, 1), (3, 2)):
            idx = (pl.ds(lo, n), pl.ds(r0, 8), pl.ds(c0, 1024))
            for m, w in enumerate((awq_hbm, bwq_hbm)):
                pltpu.make_async_copy(w.at[idx], wq_v.at[(m, *idx)], sem_wq).start(priority=m)

    def issue_kv(src, g, key0, units, unit0, piece0):
        for s in range(PPU // SPU):
            where = []
            for c in range(2):
                p = piece0 + s
                if c == 0:
                    p = (p + units * PPU - SKEW) % (units * PPU)
                where.append((
                    (unit0 + p // PPU) % N_SLOT,
                    pl.multiple_of((p % PPU) * PIECE, PIECE),
                    pl.multiple_of(key0 + p * PIECE, PIECE),
                ))
            for i in range(0, OCT, 2):
                for c, (slot, r0, k0) in enumerate(where):
                    pltpu.make_async_copy(
                        src.at[2 * g + c, pl.ds(i, 2), pl.ds(k0, PIECE)],
                        kv_v.at[slot, c, pl.ds(i, 2), pl.ds(r0, PIECE)],
                        sem_kv.at[slot],
                    ).start(priority=c)

    def issue_step(n):
        g, t = n // (2 * PASS), n % (2 * PASS)
        for src, key0, units, w in (
            (bk_hbm, 0, NB, 0),
            (ak_hbm, SK - WIN, 1, NB),
            (bv_hbm, 0, NB, NU),
            (av_hbm, SK - WIN, 1, NU + NB),
        ):

            @pl.when(jnp.logical_and(t >= SPU * w, t < SPU * (w + units)))
            def _(src=src, key0=key0, units=units, w=w):
                issue_kv(src, g, key0, units, g * 2 * NU + w, (t - SPU * w) * (PPU // SPU))

    def copy_wo(g, i, r0, branch_b_sem):
        rows = pl.ds(r0, WO_ROWS)
        for m, w in enumerate((awo_hbm, bwo_hbm)):
            sem = sem_wo.at[m, branch_b_sem if m else i]
            pltpu.make_async_copy(w.at[g, i, rows], wo_v.at[m, g, i, rows], sem).start(priority=m)

    def issue_wo(i):
        for r0 in range(0, DH, WO_ROWS):
            for g in range(N_OCT):
                copy_wo(g, i, r0, i)

    def issue_wo_last():
        for g in range(N_OCT):
            for r0 in range(0, DH, WO_ROWS):
                copy_wo(g, OCT - 1, r0, OCT - 1 + g)

    def q_proj(g):
        x = x_v[...].astype(jnp.float32)
        rows = lax.broadcasted_iota(jnp.int32, (B * OCT, D), 0)
        xs = jnp.where(rows < OCT, x[0:1], x[1:2]).astype(jnp.bfloat16)
        c0 = pl.multiple_of(g * OCT * DH, OCT * DH)

        def branch(m, _):
            w = wq_v[m, :, :, pl.ds(c0, OCT * DH)].reshape(D, OCT * DH)
            r = jnp.dot(xs, w, preferred_element_type=jnp.float32)
            for b in range(B):
                rb = r[b * OCT : (b + 1) * OCT]
                q = rb[:, 0:DH]
                for i in range(1, OCT):
                    q = jnp.where(row == i, rb[:, i * DH : (i + 1) * DH], q)
                q_scr[m, b * N_OCT + g] = q

        lax.fori_loop(0, 2, branch, None)

    def scores(g, w, j, slot):
        m = jnp.where(w == NB, 0, 1)
        rows = lax.broadcasted_iota(jnp.int32, (OCT, KU), 0)
        for c in range(2):
            q = q_scr[m, 2 * g + c].astype(jnp.bfloat16)
            for i in (2 * j, 2 * j + 1):
                s = lax.dot_general(q, kv_v[slot, c, i], _NT, preferred_element_type=jnp.float32)
                pltpu.store(s_scr.at[c, w], s, mask=rows == i)

    def softmax():
        for c in range(2):
            for m, lo, n in ((0, NB, 1), (1, 0, NB)):
                s = s_scr[c, lo : lo + n] * SCALE
                e = jnp.exp(s - jnp.max(jnp.max(s, axis=0), axis=-1, keepdims=True))
                l = jnp.sum(jnp.sum(e, axis=0), axis=-1, keepdims=True)
                l_scr[m, c] = jnp.broadcast_to(l, (OCT, DH))
                p_scr[c, lo : lo + n] = e.astype(jnp.bfloat16)
        acc_scr[...] = jnp.zeros_like(acc_scr)

    def weighted_values(w, j, slot):
        m = jnp.where(w == NB, 0, 1)
        for c in range(2):
            acc = acc_scr[m, c]
            for i in (2 * j, 2 * j + 1):
                r = jnp.dot(p_scr[c, w], kv_v[slot, c, i], preferred_element_type=jnp.float32)
                acc = acc + jnp.where(row == i, r, 0.0)
            acc_scr[m, c] = acc

    def normalize(g):
        for c in range(2):
            octet = 2 * g + c
            for m in range(2):
                o = acc_scr[m, c] / l_scr[m, c]
                for i in range(OCT):
                    o_scr[m, octet % N_OCT, i, pl.ds(octet // N_OCT, 1), :] = o[i : i + 1]

    def project(m, g, i):
        o = o_scr[m, g, i].astype(jnp.bfloat16)
        return jnp.dot(o, wo_v[m, g, i], preferred_element_type=jnp.float32)

    def add_heads(m, i, acc):
        wait_all(wo_v.at[m, :, i], sem_wo.at[m, i])
        for g in range(N_OCT):
            acc = acc + project(m, g, i)
        return acc

    copy_x = pltpu.make_async_copy(x_hbm, x_v, sem_small.at[0])
    copy_gw = pltpu.make_async_copy(gw_hbm, gw_v, sem_small.at[1])
    lax.fori_loop(0, (D // WQ_SEG // 8) * 4, issue_wq, None)
    copy_x.start()
    copy_gw.start()
    s_scr[...] = jnp.zeros_like(s_scr)
    o_scr[...] = jnp.zeros_like(o_scr)

    def step(k, _):
        pl.when(k < N_STEP)(lambda: issue_step(k))
        pl.when(k >= N_STEP)(lambda: issue_wo(k - N_STEP))

        @pl.when(k == 1)
        def _():
            copy_x.wait()
            copy_gw.wait()
            wait_all(wq_v, sem_wq)

        pl.when(jnp.logical_and(k >= 1, k <= N_OCT))(lambda: q_proj(k - 1))

        @pl.when(k >= AHEAD)
        def _():
            n = k - AHEAD
            g, t, j = n // (2 * PASS), n % (2 * PASS), n % SPU
            slot = (n // SPU) % N_SLOT
            pl.when(j == 0)(lambda: wait_all(kv_v.at[slot], sem_kv.at[slot]))
            pl.when(t < PASS)(lambda: scores(g, t // SPU, j, slot))
            pl.when(t == PASS - 1)(softmax)
            pl.when(t >= PASS)(lambda: weighted_values(t // SPU - NU, j, slot))
            pl.when(t == 2 * PASS - 1)(lambda: normalize(g))

    lax.fori_loop(0, N_STEP + AHEAD, step, None)

    x = x_v[...].astype(jnp.float32)
    gw = gw_v[...].astype(jnp.float32)
    logit = sum(
        jnp.sum(x[:, c * DH : (c + 1) * DH] * gw[c : c + 1], axis=-1, keepdims=True)
        for c in range(D // DH)
    )
    gate = jax.nn.sigmoid(logit)

    def out_proj(i, acc):
        pl.when(i == 3)(issue_wo_last)
        return add_heads(0, i + 1, acc[0]), add_heads(1, i, acc[1])

    zero = jnp.zeros((8, D), jnp.float32)
    acc_a, acc_b = lax.fori_loop(0, OCT - 1, out_proj, (add_heads(0, 0, zero), zero))
    part_a = gate * acc_a[0:B]

    def last_heads(g, acc):
        wait_all(wo_v.at[1, g, OCT - 1], sem_wo.at[1, OCT - 1 + g])
        acc = acc + project(1, g, OCT - 1)
        out_ref[...] = (part_a + (1.0 - gate) * acc[0:B]).astype(out_ref.dtype)
        return acc

    lax.fori_loop(0, N_OCT, last_heads, acc_b)


@jax.jit
def pallas_gated_mix__sliding_block_cached__mha_block_cached__decode_kernel(
    A_x: jax.Array,
    A_k_cache: jax.Array,
    A_v_cache: jax.Array,
    A_wq: jax.Array,
    A_wo: jax.Array,
    B_x: jax.Array,
    B_k_cache: jax.Array,
    B_v_cache: jax.Array,
    B_wq: jax.Array,
    B_wo: jax.Array,
    gate_w: jax.Array,
):
    del B_x
    assert A_k_cache.shape == B_k_cache.shape == (B, H, SK, DH) and A_x.shape == (B, 1, D)
    assert AHEAD == OCT - 1
    kv_shape = (B * N_OCT, OCT, SK, DH)
    wq_shape = (WQ_SEG, D // WQ_SEG, H * DH)
    wo_shape = (N_OCT, OCT, DH, D)
    out = pl.pallas_call(
        _kernel,
        in_specs=[pl.BlockSpec(memory_space=pltpu.HBM)] * 10,
        out_specs=pl.BlockSpec(memory_space=pltpu.VMEM),
        out_shape=jax.ShapeDtypeStruct((B, D), A_x.dtype),
        scratch_shapes=[
            pltpu.VMEM((B, D), jnp.bfloat16),
            pltpu.VMEM((D // DH, DH), jnp.bfloat16),
            pltpu.VMEM((2, *wq_shape), jnp.bfloat16),
            pltpu.VMEM((2, *wo_shape), jnp.bfloat16),
            pltpu.VMEM((N_SLOT, 2, OCT, KU, DH), jnp.bfloat16),
            pltpu.VMEM((2, B * N_OCT, OCT, DH), jnp.float32),
            pltpu.VMEM((2, NU, OCT, KU), jnp.float32),
            pltpu.VMEM((2, NU, OCT, KU), jnp.bfloat16),
            pltpu.VMEM((2, 2, OCT, DH), jnp.float32),
            pltpu.VMEM((2, 2, OCT, DH), jnp.float32),
            pltpu.VMEM((2, N_OCT, OCT, 8, DH), jnp.float32),
            pltpu.SemaphoreType.DMA((2,)),
            pltpu.SemaphoreType.DMA(()),
            pltpu.SemaphoreType.DMA((2, OCT - 1 + N_OCT)),
            pltpu.SemaphoreType.DMA((N_SLOT,)),
        ],
        compiler_params=pltpu.CompilerParams(
            vmem_limit_bytes=64 * 2**20,
            disable_bounds_checks=True,
            disable_semaphore_checks=True,
        ),
    )(
        A_x.reshape(B, D),
        gate_w.reshape(D // DH, DH),
        A_k_cache.reshape(kv_shape),
        A_v_cache.reshape(kv_shape),
        A_wq.reshape(wq_shape),
        A_wo.reshape(wo_shape),
        B_k_cache.reshape(kv_shape),
        B_v_cache.reshape(kv_shape),
        B_wq.reshape(wq_shape),
        B_wo.reshape(wo_shape),
    )
    return out.reshape(B, 1, D)
```

```python
import jax
import jax.numpy as jnp
from jax import lax
from jax.experimental import pallas as pl
from jax.experimental.pallas import tpu as pltpu

B, D, H, DH, SK = 2, 640, 32, 128, 4096
WIN = min(4096, max(256, SK // 4))
SCALE = DH**-0.5

OCT = 8
N_OCT = H // OCT
N_GROUP = B * N_OCT // 2
KU = WIN
NB = SK // KU
NU = NB + 1
SPU = 4
PASS = NU * SPU
N_STEP = N_GROUP * 2 * PASS
PIECE = 64
PPU = KU // PIECE
SKEW = 6
AHEAD = 7
Q_STEP = 3
N_SLOT = 6
WQ_SEG = 5

_NT = (((1,), (1,)), ((), ()))


def _kernel(
    x_hbm, gw_hbm, ak_hbm, av_hbm, awq_hbm, awo_hbm, bk_hbm, bv_hbm, bwq_hbm, bwo_hbm,
    out_ref,
    x_v, gw_v, wq_v, wo_v, kv_v, q_scr, s_scr, p_scr, l_scr, acc_scr, o_scr,
    sem_small, sem_wq, sem_wo, sem_kv,
):
    row = lax.broadcasted_iota(jnp.int32, (OCT, DH), 0)

    def wait_all(buf, sem):
        pltpu.make_async_copy(buf, buf, sem).wait()

    def issue_wq(k, _):
        r0 = pl.multiple_of((k >> 2) * 8, 8)
        c0 = pl.multiple_of((k & 3) * 1024, 1024)
        for lo, n in ((0, 2), (2, 1), (3, 2)):
            idx = (pl.ds(lo, n), pl.ds(r0, 8), pl.ds(c0, 1024))
            for m, w in enumerate((awq_hbm, bwq_hbm)):
                pltpu.make_async_copy(w.at[idx], wq_v.at[(m, *idx)], sem_wq).start(priority=m)

    def issue_kv(src, g, key0, units, unit0, piece0):
        for s in range(PPU // SPU):
            where = []
            for c in range(2):
                p = piece0 + s
                if c == 0:
                    p = (p + units * PPU - SKEW) % (units * PPU)
                where.append((
                    (unit0 + p // PPU) % N_SLOT,
                    pl.multiple_of((p % PPU) * PIECE, PIECE),
                    pl.multiple_of(key0 + p * PIECE, PIECE),
                ))
            for i in range(0, OCT, 2):
                for c, (slot, r0, k0) in enumerate(where):
                    pltpu.make_async_copy(
                        src.at[2 * g + c, pl.ds(i, 2), pl.ds(k0, PIECE)],
                        kv_v.at[slot, c, pl.ds(i, 2), pl.ds(r0, PIECE)],
                        sem_kv.at[slot],
                    ).start(priority=c)

    def issue_step(n):
        g, t = n // (2 * PASS), n % (2 * PASS)
        for src, key0, units, w in (
            (bk_hbm, 0, NB, 0),
            (ak_hbm, SK - WIN, 1, NB),
            (bv_hbm, 0, NB, NU),
            (av_hbm, SK - WIN, 1, NU + NB),
        ):

            @pl.when(jnp.logical_and(t >= SPU * w, t < SPU * (w + units)))
            def _(src=src, key0=key0, units=units, w=w):
                issue_kv(src, g, key0, units, g * 2 * NU + w, (t - SPU * w) * (PPU // SPU))

    def copy_wo(m, idx, sem):
        src = (awo_hbm, bwo_hbm)[m]
        pltpu.make_async_copy(src.at[idx], wo_v.at[(m, *idx)], sem_wo.at[m, sem]).start(priority=m)

    def wo_piece(i, k):
        return pl.ds(2 * (k % 2), 2), i, pl.ds(16 * (k // 2), 16)

    def issue_wo(i):
        for k in range(16):
            for m in range(2):
                copy_wo(m, wo_piece(i, k), i)

    def issue_wo_last():
        i = OCT - 1
        for k in range(16):
            copy_wo(0, wo_piece(i, k), i)
            copy_wo(1, (k // 4, i, pl.ds(32 * (k % 4), 32)), i + k // 4)

    def q_proj(g):
        x = x_v[...].astype(jnp.float32)
        rows = lax.broadcasted_iota(jnp.int32, (B * OCT, D), 0)
        xs = jnp.where(rows < OCT, x[0:1], x[1:2]).astype(jnp.bfloat16)
        c0 = pl.multiple_of(g * OCT * DH, OCT * DH)

        def branch(m, _):
            w = wq_v[m, :, :, pl.ds(c0, OCT * DH)].reshape(D, OCT * DH)
            r = jnp.dot(xs, w, preferred_element_type=jnp.float32)
            for b in range(B):
                rb = r[b * OCT : (b + 1) * OCT]
                q = rb[:, 0:DH]
                for i in range(1, OCT):
                    q = jnp.where(row == i, rb[:, i * DH : (i + 1) * DH], q)
                q_scr[m, b * N_OCT + g] = q

        lax.fori_loop(0, 2, branch, None)

    def scores(g, w, j, slot):
        m = jnp.where(w == NB, 0, 1)
        rows = lax.broadcasted_iota(jnp.int32, (OCT, KU), 0)
        for c in range(2):
            q = q_scr[m, 2 * g + c].astype(jnp.bfloat16)
            for i in (2 * j, 2 * j + 1):
                s = lax.dot_general(q, kv_v[slot, c, i], _NT, preferred_element_type=jnp.float32)
                pltpu.store(s_scr.at[c, w], s, mask=rows == i)

    def softmax():
        for c in range(2):
            for m, lo, n in ((0, NB, 1), (1, 0, NB)):
                s = s_scr[c, lo : lo + n] * SCALE
                e = jnp.exp(s - jnp.max(jnp.max(s, axis=0), axis=-1, keepdims=True))
                l = jnp.sum(jnp.sum(e, axis=0), axis=-1, keepdims=True)
                l_scr[m, c] = jnp.broadcast_to(l, (OCT, DH))
                p_scr[c, lo : lo + n] = e.astype(jnp.bfloat16)
        acc_scr[...] = jnp.zeros_like(acc_scr)

    def weighted_values(w, j, slot):
        m = jnp.where(w == NB, 0, 1)
        for c in range(2):
            acc = acc_scr[m, c]
            for i in (2 * j, 2 * j + 1):
                r = jnp.dot(p_scr[c, w], kv_v[slot, c, i], preferred_element_type=jnp.float32)
                acc = acc + jnp.where(row == i, r, 0.0)
            acc_scr[m, c] = acc

    def normalize(g):
        for c in range(2):
            octet = 2 * g + c
            for m in range(2):
                o = acc_scr[m, c] / l_scr[m, c]
                for i in range(OCT):
                    o_scr[m, octet % N_OCT, i, pl.ds(octet // N_OCT, 1), :] = o[i : i + 1]

    def project(m, g, i):
        o = o_scr[m, g, i].astype(jnp.bfloat16)
        return jnp.dot(o, wo_v[m, g, i], preferred_element_type=jnp.float32)

    def add_heads(m, i, acc):
        wait_all(wo_v.at[m, :, i], sem_wo.at[m, i])
        for g in range(N_OCT):
            acc = acc + project(m, g, i)
        return acc

    copy_x = pltpu.make_async_copy(x_hbm, x_v, sem_small.at[0])
    copy_gw = pltpu.make_async_copy(gw_hbm, gw_v, sem_small.at[1])
    lax.fori_loop(0, (D // WQ_SEG // 8) * 4, issue_wq, None)
    copy_x.start()
    copy_gw.start()
    s_scr[...] = jnp.zeros_like(s_scr)
    o_scr[...] = jnp.zeros_like(o_scr)

    def step(k, _):
        pl.when(k < N_STEP)(lambda: issue_step(k))
        pl.when(k >= N_STEP)(lambda: issue_wo(k - N_STEP))

        @pl.when(k == Q_STEP)
        def _():
            copy_x.wait()
            copy_gw.wait()
            wait_all(wq_v, sem_wq)

        pl.when(jnp.logical_and(k >= Q_STEP, k < Q_STEP + N_OCT))(lambda: q_proj(k - Q_STEP))

        @pl.when(k >= AHEAD)
        def _():
            n = k - AHEAD
            g, t, j = n // (2 * PASS), n % (2 * PASS), n % SPU
            slot = (n // SPU) % N_SLOT
            pl.when(j == 0)(lambda: wait_all(kv_v.at[slot], sem_kv.at[slot]))
            pl.when(t < PASS)(lambda: scores(g, t // SPU, j, slot))
            pl.when(t == PASS - 1)(softmax)
            pl.when(t >= PASS)(lambda: weighted_values(t // SPU - NU, j, slot))
            pl.when(t == 2 * PASS - 1)(lambda: normalize(g))

    lax.fori_loop(0, N_STEP + AHEAD, step, None)

    x = x_v[...].astype(jnp.float32)
    gw = gw_v[...].astype(jnp.float32)
    logit = sum(
        jnp.sum(x[:, c * DH : (c + 1) * DH] * gw[c : c + 1], axis=-1, keepdims=True)
        for c in range(D // DH)
    )
    gate = jax.nn.sigmoid(logit)

    def out_proj(i, acc):
        pl.when(i == 3)(issue_wo_last)
        return add_heads(0, i + 1, acc[0]), add_heads(1, i, acc[1])

    zero = jnp.zeros((8, D), jnp.float32)
    acc_a, acc_b = lax.fori_loop(0, OCT - 1, out_proj, (add_heads(0, 0, zero), zero))
    part_a = gate * acc_a[0:B]

    def last_heads(g, acc):
        wait_all(wo_v.at[1, g, OCT - 1], sem_wo.at[1, OCT - 1 + g])
        acc = acc + project(1, g, OCT - 1)
        out_ref[...] = (part_a + (1.0 - gate) * acc[0:B]).astype(out_ref.dtype)
        return acc

    lax.fori_loop(0, N_OCT, last_heads, acc_b)


@jax.jit
def pallas_gated_mix__sliding_block_cached__mha_block_cached__decode_kernel(
    A_x: jax.Array,
    A_k_cache: jax.Array,
    A_v_cache: jax.Array,
    A_wq: jax.Array,
    A_wo: jax.Array,
    B_x: jax.Array,
    B_k_cache: jax.Array,
    B_v_cache: jax.Array,
    B_wq: jax.Array,
    B_wo: jax.Array,
    gate_w: jax.Array,
):
    del B_x
    assert A_k_cache.shape == B_k_cache.shape == (B, H, SK, DH) and A_x.shape == (B, 1, D)
    assert AHEAD == OCT - 1 and Q_STEP + N_OCT <= AHEAD
    kv_shape = (B * N_OCT, OCT, SK, DH)
    wq_shape = (WQ_SEG, D // WQ_SEG, H * DH)
    wo_shape = (N_OCT, OCT, DH, D)
    out = pl.pallas_call(
        _kernel,
        in_specs=[pl.BlockSpec(memory_space=pltpu.HBM)] * 10,
        out_specs=pl.BlockSpec(memory_space=pltpu.VMEM),
        out_shape=jax.ShapeDtypeStruct((B, D), A_x.dtype),
        scratch_shapes=[
            pltpu.VMEM((B, D), jnp.bfloat16),
            pltpu.VMEM((D // DH, DH), jnp.bfloat16),
            pltpu.VMEM((2, *wq_shape), jnp.bfloat16),
            pltpu.VMEM((2, *wo_shape), jnp.bfloat16),
            pltpu.VMEM((N_SLOT, 2, OCT, KU, DH), jnp.bfloat16),
            pltpu.VMEM((2, B * N_OCT, OCT, DH), jnp.float32),
            pltpu.VMEM((2, NU, OCT, KU), jnp.float32),
            pltpu.VMEM((2, NU, OCT, KU), jnp.bfloat16),
            pltpu.VMEM((2, 2, OCT, DH), jnp.float32),
            pltpu.VMEM((2, 2, OCT, DH), jnp.float32),
            pltpu.VMEM((2, N_OCT, OCT, 8, DH), jnp.float32),
            pltpu.SemaphoreType.DMA((2,)),
            pltpu.SemaphoreType.DMA(()),
            pltpu.SemaphoreType.DMA((2, OCT - 1 + N_OCT)),
            pltpu.SemaphoreType.DMA((N_SLOT,)),
        ],
        compiler_params=pltpu.CompilerParams(
            vmem_limit_bytes=64 * 2**20,
            disable_bounds_checks=True,
            disable_semaphore_checks=True,
        ),
    )(
        A_x.reshape(B, D),
        gate_w.reshape(D // DH, DH),
        A_k_cache.reshape(kv_shape),
        A_v_cache.reshape(kv_shape),
        A_wq.reshape(wq_shape),
        A_wo.reshape(wo_shape),
        B_k_cache.reshape(kv_shape),
        B_v_cache.reshape(kv_shape),
        B_wq.reshape(wq_shape),
        B_wo.reshape(wo_shape),
    )
    return out.reshape(B, 1, D)
```
